```python
import os as _os
_os.environ.setdefault("JAX_PLATFORMS", "cpu")
import jax
import jax.numpy as jnp

def _softmax(x, axis=-1):
    return jax.nn.softmax(x, axis=axis)
def _gelu(x):
    return jax.nn.gelu(x, approximate=True)
def _silu(x):
    return jax.nn.silu(x)
def _sigmoid(x):
    return jax.nn.sigmoid(x)
def _layernorm(x, axis=-1, eps=1e-5):
    m = jnp.mean(x, axis=axis, keepdims=True)
    v = jnp.var(x, axis=axis, keepdims=True)
    return (x - m) / jnp.sqrt(v + eps)
def _scatter_add(tgt, idx, src, axis=0):
    return tgt.at[idx].add(src)
def _segment_sum(src, seg, n):
    return jax.ops.segment_sum(src, seg, n)
class _Rng:
    def __init__(self, key):
        self._k = key
    def _next(self):
        self._k, sub = jax.random.split(self._k)
        return sub
    def normal(self, shape):
        return jax.random.normal(self._next(), shape, dtype=jnp.bfloat16)
    def randint(self, lo, hi, shape):
        return jax.random.randint(self._next(), shape, lo, hi, dtype=jnp.int32)
    def uniform(self, shape, lo=0.0, hi=1.0):
        return jax.random.uniform(self._next(), shape, jnp.bfloat16, lo, hi)
    def permutation(self, n):
        return jax.random.permutation(self._next(), n)


kernel_name = 'standalone__gqa_block_cached__near_ridge'

def setup_inputs():
    _rng = _Rng(jax.random.key(int.from_bytes(__import__("os").urandom(4), "little")))
    _w = (lambda a: (lambda t: t.astype(jnp.bfloat16) if jnp.issubdtype(t.dtype, jnp.floating) else t)(jnp.asarray(a)))
    B, Sq, D = 8, 64, 512
    Hq, Hkv, Sk, Dh = 32, 8, 64, 128
    assert Hq % Hkv == 0, (Hq, Hkv)
    return {
        "x": _w((lambda *s: _rng.normal(s) * 0.8)(B, Sq, D)),
        "k_cache": _w((lambda *s: _rng.normal(s) * 0.8)(B, Hkv, Sk, Dh)),
        "v_cache": _w((lambda *s: _rng.normal(s) * 0.05)(B, Hkv, Sk, Dh)),
        "wq": _w((lambda *s: _rng.normal(s) * 0.8)(D, Hq * Dh) * (D ** -0.5)),
        "wo": _w((lambda *s: _rng.normal(s) * 0.05)(Hq * Dh, D) * ((Hq * Dh) ** -0.5)),
    }

def reference(x, k_cache, v_cache, wq, wo):
    B, Sq, D = x.shape
    Hq, Dh = 32, 128
    Hkv = k_cache.shape[1]
    rep = Hq // Hkv
    q = (lambda x, *d: x.transpose(*d))((x @ wq).reshape(B, Sq, Hq, Dh), 0, 2, 1, 3)
    k = jnp.repeat(k_cache, rep, axis=1)
    v = jnp.repeat(v_cache, rep, axis=1)
    scores = jnp.einsum("bhqd,bhkd->bhqk", q, k) * (Dh ** -0.5)
    p = _softmax(scores, axis=-1)
    o = jnp.einsum("bhqk,bhkd->bhqd", p, v)
    return (lambda x, *d: x.transpose(*d))(o, 0, 2, 1, 3).reshape(B, Sq, Hq * Dh) @ wo
```

```python
import functools

import jax
import jax.numpy as jnp
import jax.experimental.pallas as pl
import jax.experimental.pallas.tpu as pltpu


def _kernel(x_ref, k_ref, v_ref, wq_ref, wo_ref, o_ref, acc_ref, *, B, Sq, rep, Dh):
    g = pl.program_id(0)
    ng = pl.num_programs(0)
    scale = Dh ** -0.5

    q = jnp.dot(x_ref[...], wq_ref[...], preferred_element_type=jnp.float32)
    q = q.astype(jnp.bfloat16)

    o_parts = []
    for b in range(B):
        qb = q[b * Sq:(b + 1) * Sq, :]
        qs = jnp.concatenate(
            [qb[:, h * Dh:(h + 1) * Dh] for h in range(rep)], axis=0)
        kb = k_ref[b, 0]
        vb = v_ref[b, 0]
        s = jax.lax.dot_general(
            qs, kb, (((1,), (1,)), ((), ())),
            preferred_element_type=jnp.float32) * scale
        m = jnp.max(s, axis=-1, keepdims=True)
        p = jnp.exp(s - m)
        l = jnp.sum(p, axis=-1, keepdims=True)
        p = (p / l).astype(jnp.bfloat16)
        ob = jnp.dot(p, vb, preferred_element_type=jnp.float32).astype(jnp.bfloat16)
        ob = jnp.concatenate(
            [ob[h * Sq:(h + 1) * Sq, :] for h in range(rep)], axis=1)
        o_parts.append(ob)
    o = jnp.concatenate(o_parts, axis=0)

    part = jnp.dot(o, wo_ref[...], preferred_element_type=jnp.float32)

    @pl.when(g == 0)
    def _():
        acc_ref[...] = part

    @pl.when(g > 0)
    def _():
        acc_ref[...] += part

    @pl.when(g == ng - 1)
    def _():
        o_ref[...] = acc_ref[...].astype(o_ref.dtype)


@jax.jit
def pallas_standalone__gqa_block_cached__near_ridge_kernel(
    x: jax.Array,
    k_cache: jax.Array,
    v_cache: jax.Array,
    wq: jax.Array,
    wo: jax.Array,
):
    B, Sq, D = x.shape
    _, Hkv, Sk, Dh = k_cache.shape
    Hq = wq.shape[1] // Dh
    rep = Hq // Hkv
    M = B * Sq
    G = rep * Dh

    x2 = x.reshape(M, D)

    kernel = functools.partial(_kernel, B=B, Sq=Sq, rep=rep, Dh=Dh)
    out = pl.pallas_call(
        kernel,
        grid=(Hkv,),
        in_specs=[
            pl.BlockSpec((M, D), lambda g: (0, 0)),
            pl.BlockSpec((B, 1, Sk, Dh), lambda g: (0, g, 0, 0)),
            pl.BlockSpec((B, 1, Sk, Dh), lambda g: (0, g, 0, 0)),
            pl.BlockSpec((D, G), lambda g: (0, g)),
            pl.BlockSpec((G, D), lambda g: (g, 0)),
        ],
        out_specs=pl.BlockSpec((M, D), lambda g: (0, 0)),
        out_shape=jax.ShapeDtypeStruct((M, D), x.dtype),
        scratch_shapes=[pltpu.VMEM((M, D), jnp.float32)],
        compiler_params=pltpu.CompilerParams(
            dimension_semantics=("arbitrary",),
            vmem_limit_bytes=64 * 1024 * 1024,
        ),
    )(x2, k_cache, v_cache, wq, wo)
    return out.reshape(B, Sq, D)
```

```python
import functools

import jax
import jax.numpy as jnp
import jax.experimental.pallas as pl
import jax.experimental.pallas.tpu as pltpu

LANE = 128


def _body(refs, *, do_a, do_b, do_c, B, Sq, rep, Dh):
    (x_ref, wq_ref, q_out, k_ref, v_ref, q_in, o_out, o_in, wo_ref, acc_ref) = refs
    scale = Dh ** -0.5

    def chunk_a(j):
        sl = slice(j * LANE, (j + 1) * LANE)
        q = jnp.dot(x_ref[...], wq_ref[:, sl], preferred_element_type=jnp.float32)
        q_out[:, sl] = q.astype(q_out.dtype)

    def chunk_c(j):
        sl = slice(j * LANE, (j + 1) * LANE)
        acc_ref[:, sl] += jnp.dot(o_in[...], wo_ref[:, sl],
                                  preferred_element_type=jnp.float32)

    chunks = []
    na = (rep * Dh) // LANE
    nc = acc_ref.shape[1] // LANE
    for j in range(max(na, nc)):
        if do_a and j < na:
            chunks.append(functools.partial(chunk_a, j))
        if do_c and j < nc:
            chunks.append(functools.partial(chunk_c, j))

    if not do_b:
        for c in chunks:
            c()
        return

    n = len(chunks)
    for b in range(B):
        qs = jnp.concatenate(
            [q_in[b * Sq:(b + 1) * Sq, h * Dh:(h + 1) * Dh] for h in range(rep)],
            axis=0)
        kb = k_ref[b, 0]
        vb = v_ref[b, 0]
        sT = jax.lax.dot_general(
            kb, qs, (((1,), (1,)), ((), ())),
            preferred_element_type=jnp.float32) * scale
        for c in chunks[b * n // B:(b + 1) * n // B]:
            c()
        m = jnp.max(sT, axis=0, keepdims=True)
        pT = jnp.exp(sT - m)
        l = jnp.sum(pT, axis=0, keepdims=True)
        pT = (pT / l).astype(jnp.bfloat16)
        ob = jax.lax.dot_general(
            pT, vb, (((0,), (0,)), ((), ())),
            preferred_element_type=jnp.float32).astype(o_out.dtype)
        for h in range(rep):
            o_out[b * Sq:(b + 1) * Sq, h * Dh:(h + 1) * Dh] = ob[h * Sq:(h + 1) * Sq, :]


def _kernel(x_ref, k_ref, v_ref, wq_ref, wo_ref, out_ref,
            q0, q1, o0, o1, acc_ref, *, B, Sq, rep, Dh, Hkv):
    t = pl.program_id(0)
    body = functools.partial(_body, B=B, Sq=Sq, rep=rep, Dh=Dh)
    even = (t % 2) == 0
    steady = jnp.logical_and(t >= 2, t < Hkv)

    def refs(q_out, q_in, o_out, o_in):
        return (x_ref, wq_ref, q_out, k_ref, v_ref, q_in, o_out, o_in, wo_ref, acc_ref)

    @pl.when(t == 0)
    def _():
        acc_ref[...] = jnp.zeros(acc_ref.shape, acc_ref.dtype)
        body(refs(q0, None, None, None), do_a=True, do_b=False, do_c=False)

    @pl.when(t == 1)
    def _():
        body(refs(q1, q0, o0, None), do_a=True, do_b=True, do_c=False)

    @pl.when(jnp.logical_and(steady, even))
    def _():
        body(refs(q0, q1, o1, o0), do_a=True, do_b=True, do_c=True)

    @pl.when(jnp.logical_and(steady, jnp.logical_not(even)))
    def _():
        body(refs(q1, q0, o0, o1), do_a=True, do_b=True, do_c=True)

    @pl.when(t == Hkv)
    def _():
        body(refs(None, q1, o1, o0), do_a=False, do_b=True, do_c=True)

    @pl.when(t == Hkv + 1)
    def _():
        body(refs(None, None, None, o1), do_a=False, do_b=False, do_c=True)
        out_ref[...] = acc_ref[...].astype(out_ref.dtype)


@jax.jit
def pallas_standalone__gqa_block_cached__near_ridge_kernel(x, k_cache, v_cache, wq, wo):
    B, Sq, D = x.shape
    _, Hkv, Sk, Dh = k_cache.shape
    Hq = wq.shape[1] // Dh
    rep = Hq // Hkv
    M = B * Sq
    G = rep * Dh
    assert Hkv % 2 == 0

    x2 = x.reshape(M, D)

    kernel = functools.partial(_kernel, B=B, Sq=Sq, rep=rep, Dh=Dh, Hkv=Hkv)
    last = Hkv - 1
    out = pl.pallas_call(
        kernel,
        grid=(Hkv + 2,),
        in_specs=[
            pl.BlockSpec((M, D), lambda t: (0, 0)),
            pl.BlockSpec((B, 1, Sk, Dh), lambda t: (0, jnp.clip(t - 1, 0, last), 0, 0)),
            pl.BlockSpec((B, 1, Sk, Dh), lambda t: (0, jnp.clip(t - 1, 0, last), 0, 0)),
            pl.BlockSpec((D, G), lambda t: (0, jnp.minimum(t, last))),
            pl.BlockSpec((G, D), lambda t: (jnp.clip(t - 2, 0, last), 0)),
        ],
        out_specs=pl.BlockSpec((M, D), lambda t: (0, 0)),
        out_shape=jax.ShapeDtypeStruct((M, D), x.dtype),
        scratch_shapes=[
            pltpu.VMEM((M, G), jnp.bfloat16),
            pltpu.VMEM((M, G), jnp.bfloat16),
            pltpu.VMEM((M, G), jnp.bfloat16),
            pltpu.VMEM((M, G), jnp.bfloat16),
            pltpu.VMEM((M, D), jnp.float32),
        ],
        compiler_params=pltpu.CompilerParams(
            dimension_semantics=("arbitrary",),
            vmem_limit_bytes=64 * 1024 * 1024,
        ),
    )(x2, k_cache, v_cache, wq, wo)
    return out.reshape(B, Sq, D)
```

```python
import functools

import jax
import jax.numpy as jnp
import jax.experimental.pallas as pl
import jax.experimental.pallas.tpu as pltpu

LANE = 128


def _body(refs, g, *, do_a, do_b, do_c, final, B, Sq, rep, Dh):
    (x_v, wq_v, q_out, k_v, v_v, q_in, o_out, o_in, wo_v, acc_ref, outb, out_hbm,
     sems, out_sem0) = refs
    scale = Dh ** -0.5

    def chunk_a(j):
        sl = slice(j * LANE, (j + 1) * LANE)
        q = jnp.dot(x_v[...], wq_v[g, :, sl], preferred_element_type=jnp.float32)
        q_out[:, sl] = q.astype(q_out.dtype)

    def chunk_c(j):
        sl = slice(j * LANE, (j + 1) * LANE)
        r = acc_ref[:, sl] + jnp.dot(o_in[...], wo_v[g - 2, :, sl],
                                     preferred_element_type=jnp.float32)
        if final:
            outb[:, sl] = r.astype(outb.dtype)
            pltpu.make_async_copy(outb.at[:, sl], out_hbm.at[:, sl],
                                  sems.at[out_sem0 + j]).start()
        else:
            acc_ref[:, sl] = r

    chunks = []
    na = (rep * Dh) // LANE
    nc = acc_ref.shape[1] // LANE
    for j in range(max(na, nc)):
        if do_a and j < na:
            chunks.append(functools.partial(chunk_a, j))
        if do_c and j < nc:
            chunks.append(functools.partial(chunk_c, j))

    if not do_b:
        for c in chunks:
            c()
        return

    n = len(chunks)
    for b in range(B):
        qs = jnp.concatenate(
            [q_in[b * Sq:(b + 1) * Sq, h * Dh:(h + 1) * Dh] for h in range(rep)],
            axis=0)
        kb = k_v[g - 1, b]
        vb = v_v[g - 1, b]
        sT = jax.lax.dot_general(
            kb, qs, (((1,), (1,)), ((), ())),
            preferred_element_type=jnp.float32) * scale
        for c in chunks[b * n // B:(b + 1) * n // B]:
            c()
        m = jnp.max(sT, axis=0, keepdims=True)
        pT = jnp.exp(sT - m)
        l = jnp.sum(pT, axis=0, keepdims=True)
        pT = (pT / l).astype(jnp.bfloat16)
        ob = jax.lax.dot_general(
            pT, vb, (((0,), (0,)), ((), ())),
            preferred_element_type=jnp.float32).astype(o_out.dtype)
        for h in range(rep):
            o_out[b * Sq:(b + 1) * Sq, h * Dh:(h + 1) * Dh] = ob[h * Sq:(h + 1) * Sq, :]


def _kernel(x_hbm, k_hbm, v_hbm, wq_hbm, wo_hbm, out_hbm,
            x_v, k_v, v_v, wq_v, wo_v, q0, q1, o0, o1, acc_ref, outb, sems,
            *, B, Sq, rep, Dh, Hkv):
    t = pl.program_id(0)
    G = rep * Dh
    nout = outb.shape[1] // LANE
    S_X, S_WQ, S_WO, S_K, S_V = 0, 1, 1 + Hkv, 1 + 2 * Hkv, 1 + 3 * Hkv
    S_OUT = 1 + 4 * Hkv

    def cp_x():
        return pltpu.make_async_copy(x_hbm, x_v, sems.at[S_X])

    def cp_wq(g):
        return pltpu.make_async_copy(wq_hbm.at[:, pl.ds(g * G, G)], wq_v.at[g],
                                     sems.at[S_WQ + g])

    def cp_wo(g):
        return pltpu.make_async_copy(wo_hbm.at[pl.ds(g * G, G), :], wo_v.at[g],
                                     sems.at[S_WO + g])

    def cp_k(g):
        return pltpu.make_async_copy(k_hbm.at[:, g], k_v.at[g], sems.at[S_K + g])

    def cp_v(g):
        return pltpu.make_async_copy(v_hbm.at[:, g], v_v.at[g], sems.at[S_V + g])

    body = functools.partial(_body, B=B, Sq=Sq, rep=rep, Dh=Dh)

    def refs(q_out, q_in, o_out, o_in):
        return (x_v, wq_v, q_out, k_v, v_v, q_in, o_out, o_in, wo_v, acc_ref, outb,
                out_hbm, sems, S_OUT)

    even = (t % 2) == 0
    steady = jnp.logical_and(t >= 2, t < Hkv)

    @pl.when(t == 0)
    def _():
        cp_x().start()
        cp_wq(0).start()
        for g in range(Hkv):
            cp_k(g).start()
            cp_v(g).start()
            if g + 1 < Hkv:
                cp_wq(g + 1).start()
            cp_wo(g).start()
        acc_ref[...] = jnp.zeros(acc_ref.shape, acc_ref.dtype)
        cp_x().wait()
        cp_wq(0).wait()
        body(refs(q0, None, None, None), 0, do_a=True, do_b=False, do_c=False,
             final=False)

    @pl.when(t == 1)
    def _():
        cp_wq(1).wait()
        cp_k(0).wait()
        cp_v(0).wait()
        body(refs(q1, q0, o0, None), 1, do_a=True, do_b=True, do_c=False, final=False)

    @pl.when(steady)
    def _():
        cp_wq(t).wait()
        cp_k(t - 1).wait()
        cp_v(t - 1).wait()
        cp_wo(t - 2).wait()

    @pl.when(jnp.logical_and(steady, even))
    def _():
        body(refs(q0, q1, o1, o0), t, do_a=True, do_b=True, do_c=True, final=False)

    @pl.when(jnp.logical_and(steady, jnp.logical_not(even)))
    def _():
        body(refs(q1, q0, o0, o1), t, do_a=True, do_b=True, do_c=True, final=False)

    @pl.when(t == Hkv)
    def _():
        cp_k(Hkv - 1).wait()
        cp_v(Hkv - 1).wait()
        cp_wo(Hkv - 2).wait()
        body(refs(None, q1, o1, o0), Hkv, do_a=False, do_b=True, do_c=True, final=False)

    @pl.when(t == Hkv + 1)
    def _():
        cp_wo(Hkv - 1).wait()
        body(refs(None, None, None, o1), Hkv + 1, do_a=False, do_b=False, do_c=True,
             final=True)
        for j in range(nout):
            sl = slice(j * LANE, (j + 1) * LANE)
            pltpu.make_async_copy(outb.at[:, sl], out_hbm.at[:, sl],
                                  sems.at[S_OUT + j]).wait()


@jax.jit
def pallas_standalone__gqa_block_cached__near_ridge_kernel(x, k_cache, v_cache, wq, wo):
    B, Sq, D = x.shape
    _, Hkv, Sk, Dh = k_cache.shape
    Hq = wq.shape[1] // Dh
    rep = Hq // Hkv
    M = B * Sq
    G = rep * Dh
    assert Hkv % 2 == 0

    x2 = x.reshape(M, D)

    kernel = functools.partial(_kernel, B=B, Sq=Sq, rep=rep, Dh=Dh, Hkv=Hkv)
    any_spec = pl.BlockSpec(memory_space=pl.ANY)
    out = pl.pallas_call(
        kernel,
        grid=(Hkv + 2,),
        in_specs=[any_spec] * 5,
        out_specs=any_spec,
        out_shape=jax.ShapeDtypeStruct((M, D), x.dtype),
        scratch_shapes=[
            pltpu.VMEM((M, D), x.dtype),
            pltpu.VMEM((Hkv, B, Sk, Dh), k_cache.dtype),
            pltpu.VMEM((Hkv, B, Sk, Dh), v_cache.dtype),
            pltpu.VMEM((Hkv, D, G), wq.dtype),
            pltpu.VMEM((Hkv, G, D), wo.dtype),
            pltpu.VMEM((M, G), jnp.bfloat16),
            pltpu.VMEM((M, G), jnp.bfloat16),
            pltpu.VMEM((M, G), jnp.bfloat16),
            pltpu.VMEM((M, G), jnp.bfloat16),
            pltpu.VMEM((M, D), jnp.float32),
            pltpu.VMEM((M, D), x.dtype),
            pltpu.SemaphoreType.DMA((1 + 4 * Hkv + D // LANE,)),
        ],
        compiler_params=pltpu.CompilerParams(
            dimension_semantics=("arbitrary",),
            vmem_limit_bytes=64 * 1024 * 1024,
        ),
    )(x2, k_cache, v_cache, wq, wo)
    return out.reshape(B, Sq, D)
```

```python
import functools

import jax
import jax.numpy as jnp
import jax.experimental.pallas as pl
import jax.experimental.pallas.tpu as pltpu

LANE = 128
SKEW = 2


def _phase(refs, g, *, do_a, do_b, do_c, final, B, Sq, rep, Dh):
    (x_v, wq_v, q_out, k_v, v_v, q_in, o_out, o_in, wo_v, acc_ref, outb, out_hbm,
     sems, out_sem0) = refs
    scale = Dh ** -0.5

    def chunk_a(j):
        sl = slice(j * LANE, (j + 1) * LANE)
        q = jnp.dot(x_v[...], wq_v[g, :, sl], preferred_element_type=jnp.float32)
        q_out[:, sl] = q.astype(q_out.dtype)

    def chunk_c(j):
        sl = slice(j * LANE, (j + 1) * LANE)
        r = acc_ref[:, sl] + jnp.dot(o_in[...], wo_v[g - 2, :, sl],
                                     preferred_element_type=jnp.float32)
        if final:
            outb[:, sl] = r.astype(outb.dtype)
            pltpu.make_async_copy(outb.at[:, sl], out_hbm.at[:, sl],
                                  sems.at[out_sem0 + j]).start()
        else:
            acc_ref[:, sl] = r

    chunks = []
    na = (rep * Dh) // LANE
    nc = acc_ref.shape[1] // LANE
    for j in range(max(na, nc)):
        if do_a and j < na:
            chunks.append(functools.partial(chunk_a, j))
        if do_c and j < nc:
            chunks.append(functools.partial(chunk_c, j))

    if not do_b:
        for c in chunks:
            c()
        return

    def scores_t(b):
        qs = jnp.concatenate(
            [q_in[b * Sq:(b + 1) * Sq, h * Dh:(h + 1) * Dh] for h in range(rep)],
            axis=0)
        return jax.lax.dot_general(
            k_v[g - 1, b], qs, (((1,), (1,)), ((), ())),
            preferred_element_type=jnp.float32) * scale

    n = len(chunks)
    pending = [scores_t(b) for b in range(min(SKEW, B))]
    for b in range(B):
        if b + SKEW < B:
            pending.append(scores_t(b + SKEW))
        s_t = pending.pop(0)
        for c in chunks[b * n // B:(b + 1) * n // B]:
            c()
        m = jnp.max(s_t, axis=0, keepdims=True)
        p_t = jnp.exp(s_t - m)
        l = jnp.sum(p_t, axis=0, keepdims=True)
        p_t = (p_t / l).astype(v_v.dtype)
        ob = jax.lax.dot_general(
            p_t, v_v[g - 1, b], (((0,), (0,)), ((), ())),
            preferred_element_type=jnp.float32).astype(o_out.dtype)
        for h in range(rep):
            o_out[b * Sq:(b + 1) * Sq, h * Dh:(h + 1) * Dh] = ob[h * Sq:(h + 1) * Sq, :]


def _kernel(x_hbm, k_hbm, v_hbm, wq_hbm, wo_hbm, out_hbm,
            x_v, k_v, v_v, wq_v, wo_v, q0, q1, o0, o1, acc_ref, outb, sems,
            *, B, Sq, rep, Dh, Hkv):
    s = pl.program_id(0)
    G = rep * Dh
    M = B * Sq
    na = G // LANE
    nout = outb.shape[1] // LANE

    S_X = 0
    S_WQ0 = S_X + 2
    S_WQ = S_WQ0 + na - 1
    S_WO = S_WQ + Hkv
    S_K = S_WO + Hkv
    S_V = S_K + Hkv
    S_OUT = S_V + Hkv

    def cp_x(i):
        rows = pl.ds(i * (M // 2), M // 2)
        return pltpu.make_async_copy(x_hbm.at[rows, :], x_v.at[rows, :], sems.at[S_X + i])

    def cp_wq0(j):
        cols = pl.ds(j * LANE, LANE)
        return pltpu.make_async_copy(wq_hbm.at[:, cols], wq_v.at[0, :, cols],
                                     sems.at[S_WQ0 + j])

    def cp_wq(g):
        return pltpu.make_async_copy(wq_hbm.at[:, pl.ds(g * G, G)], wq_v.at[g],
                                     sems.at[S_WQ + g])

    def cp_wo(g):
        return pltpu.make_async_copy(wo_hbm.at[pl.ds(g * G, G), :], wo_v.at[g],
                                     sems.at[S_WO + g])

    def cp_k(g):
        return pltpu.make_async_copy(k_hbm.at[:, g], k_v.at[g], sems.at[S_K + g])

    def cp_v(g):
        return pltpu.make_async_copy(v_hbm.at[:, g], v_v.at[g], sems.at[S_V + g])

    phase = functools.partial(_phase, B=B, Sq=Sq, rep=rep, Dh=Dh)
    q_bufs = (q0, q1)
    o_bufs = (o0, o1)

    def run(t, par, **kw):
        refs = (x_v, wq_v, q_bufs[par], k_v, v_v, q_bufs[1 - par], o_bufs[1 - par],
                o_bufs[par], wo_v, acc_ref, outb, out_hbm, sems, S_OUT)
        phase(refs, t, **kw)

    def waits(t):
        static = isinstance(t, int)
        if not static or t < Hkv:
            cp_wq(t).wait()
        if not static or t <= Hkv:
            cp_k(t - 1).wait()
            cp_v(t - 1).wait()
        if not static or t >= 2:
            cp_wo(t - 2).wait()

    full = dict(do_a=True, do_b=True, do_c=True, final=False)
    n_mid = (Hkv - 4) // 2

    @pl.when(s == 0)
    def _():
        cp_x(0).start()
        cp_wq0(0).start()
        cp_x(1).start()
        for j in range(1, na):
            cp_wq0(j).start()
        for g in range(Hkv):
            cp_k(g).start()
            cp_v(g).start()
            if g + 1 < Hkv:
                cp_wq(g + 1).start()
            cp_wo(g).start()
        acc_ref[...] = jnp.zeros(acc_ref.shape, acc_ref.dtype)

        lo, hi, al = slice(0, M // 2), slice(M // 2, M), slice(0, M)
        steps = (
            ((cp_x(0), cp_wq0(0)), ((lo, 0),)),
            ((cp_x(1), cp_wq0(1)), ((hi, 0), (al, 1))),
            (tuple(cp_wq0(j) for j in range(2, na)),
             tuple((al, j) for j in range(2, na))),
        )
        for copies, pieces in steps:
            for c in copies:
                c.wait()
            for rows, j in pieces:
                sl = slice(j * LANE, (j + 1) * LANE)
                q0[rows, sl] = jnp.dot(
                    x_v[rows, :], wq_v[0, :, sl],
                    preferred_element_type=jnp.float32).astype(q0.dtype)

        waits(1)
        run(1, 1, do_a=True, do_b=True, do_c=False, final=False)
        waits(2)
        run(2, 0, **full)

    @pl.when(jnp.logical_and(s >= 1, s <= n_mid))
    def _():
        t = 2 * s + 1
        waits(t)
        waits(t + 1)
        run(t, 1, **full)
        run(t + 1, 0, **full)

    @pl.when(s == n_mid + 1)
    def _():
        for t in (Hkv - 1, Hkv, Hkv + 1):
            waits(t)
        run(Hkv - 1, 1, **full)
        run(Hkv, 0, do_a=False, do_b=True, do_c=True, final=False)
        run(Hkv + 1, 1, do_a=False, do_b=False, do_c=True, final=True)
        for j in range(nout):
            sl = slice(j * LANE, (j + 1) * LANE)
            pltpu.make_async_copy(outb.at[:, sl], out_hbm.at[:, sl],
                                  sems.at[S_OUT + j]).wait()


@jax.jit
def pallas_standalone__gqa_block_cached__near_ridge_kernel(
    x: jax.Array,
    k_cache: jax.Array,
    v_cache: jax.Array,
    wq: jax.Array,
    wo: jax.Array,
):
    B, Sq, D = x.shape
    _, Hkv, Sk, Dh = k_cache.shape
    Hq = wq.shape[1] // Dh
    rep = Hq // Hkv
    M = B * Sq
    G = rep * Dh
    assert Hkv % 2 == 0 and Hkv >= 4 and M % 2 == 0
    assert G % LANE == 0 and D % LANE == 0 and G // LANE >= 2

    x2 = x.reshape(M, D)

    kernel = functools.partial(_kernel, B=B, Sq=Sq, rep=rep, Dh=Dh, Hkv=Hkv)
    any_spec = pl.BlockSpec(memory_space=pl.ANY)
    n_sem = 2 + (G // LANE - 1) + 4 * Hkv + D // LANE
    out = pl.pallas_call(
        kernel,
        grid=((Hkv - 4) // 2 + 2,),
        in_specs=[any_spec] * 5,
        out_specs=any_spec,
        out_shape=jax.ShapeDtypeStruct((M, D), x.dtype),
        scratch_shapes=[
            pltpu.VMEM((M, D), x.dtype),
            pltpu.VMEM((Hkv, B, Sk, Dh), k_cache.dtype),
            pltpu.VMEM((Hkv, B, Sk, Dh), v_cache.dtype),
            pltpu.VMEM((Hkv, D, G), wq.dtype),
            pltpu.VMEM((Hkv, G, D), wo.dtype),
            pltpu.VMEM((M, G), x.dtype),
            pltpu.VMEM((M, G), x.dtype),
            pltpu.VMEM((M, G), x.dtype),
            pltpu.VMEM((M, G), x.dtype),
            pltpu.VMEM((M, D), jnp.float32),
            pltpu.VMEM((M, D), x.dtype),
            pltpu.SemaphoreType.DMA((n_sem,)),
        ],
        compiler_params=pltpu.CompilerParams(
            dimension_semantics=("arbitrary",),
            vmem_limit_bytes=64 * 1024 * 1024,
        ),
    )(x2, k_cache, v_cache, wq, wo)
    return out.reshape(B, Sq, D)
```

```python
import functools

import jax
import jax.numpy as jnp
import jax.experimental.pallas as pl
import jax.experimental.pallas.tpu as pltpu

LANE = 128
SKEW = 2


def _phase(refs, g, *, do_a, do_b, do_c, final, B, Sq, rep, Dh):
    (x_v, wq_v, q_out, k_v, v_v, q_in, o_out, o_in, wo_v, acc_ref, outb, out_hbm,
     sems, out_sem0) = refs
    scale = Dh ** -0.5

    def chunk_a(j):
        sl = slice(j * LANE, (j + 1) * LANE)
        q = jnp.dot(x_v[...], wq_v[g, :, sl], preferred_element_type=jnp.float32)
        q_out[:, sl] = q.astype(q_out.dtype)

    def chunk_c(j):
        sl = slice(j * LANE, (j + 1) * LANE)
        r = acc_ref[:, sl] + jnp.dot(o_in[...], wo_v[g - 2, :, sl],
                                     preferred_element_type=jnp.float32)
        if final:
            outb[:, sl] = r.astype(outb.dtype)
            pltpu.make_async_copy(outb.at[:, sl], out_hbm.at[:, sl],
                                  sems.at[out_sem0 + j]).start()
        else:
            acc_ref[:, sl] = r

    chunks = []
    na = (rep * Dh) // LANE
    nc = acc_ref.shape[1] // LANE
    for j in range(max(na, nc)):
        if do_a and j < na:
            chunks.append(functools.partial(chunk_a, j))
        if do_c and j < nc:
            chunks.append(functools.partial(chunk_c, j))

    if not do_b:
        for c in chunks:
            c()
        return

    def scores_t(b):
        qs = jnp.concatenate(
            [q_in[b * Sq:(b + 1) * Sq, h * Dh:(h + 1) * Dh] for h in range(rep)],
            axis=0)
        return jax.lax.dot_general(
            k_v[g - 1, b], qs, (((1,), (1,)), ((), ())),
            preferred_element_type=jnp.float32) * scale

    n = len(chunks)
    slots = [[] for _ in range(B)]
    for i, c in enumerate(chunks):
        slots[(i * B) // n].append(c)

    pending = [scores_t(b) for b in range(min(SKEW, B))]
    for b in range(B):
        if b + SKEW < B:
            pending.append(scores_t(b + SKEW))
        s_t = pending.pop(0)
        for c in slots[b]:
            c()
        vb = v_v[g - 1, b]
        m = jnp.max(s_t, axis=0, keepdims=True)
        p_t = jnp.exp(s_t - m)
        l = jnp.sum(p_t, axis=0, keepdims=True)
        p_t = (p_t / l).astype(vb.dtype)
        ob = jax.lax.dot_general(
            p_t, vb, (((0,), (0,)), ((), ())),
            preferred_element_type=jnp.float32).astype(o_out.dtype)
        for h in range(rep):
            o_out[b * Sq:(b + 1) * Sq, h * Dh:(h + 1) * Dh] = ob[h * Sq:(h + 1) * Sq, :]


def _kernel(x_hbm, k_hbm, v_hbm, wq_hbm, wo_hbm, out_hbm,
            x_v, k_v, v_v, wq_v, wo_v, q0, q1, o0, o1, acc_ref, outb, sems,
            *, B, Sq, rep, Dh, Hkv):
    s = pl.program_id(0)
    G = rep * Dh
    M = B * Sq
    na = G // LANE
    nout = outb.shape[1] // LANE

    S_X = 0
    S_WQ0 = S_X + 2
    S_WQ = S_WQ0 + na - 1
    S_WO = S_WQ + Hkv
    S_K = S_WO + Hkv
    S_V = S_K + Hkv
    S_OUT = S_V + Hkv

    def cp_x(i):
        rows = pl.ds(i * (M // 2), M // 2)
        return pltpu.make_async_copy(x_hbm.at[rows, :], x_v.at[rows, :], sems.at[S_X + i])

    def cp_wq0(j):
        cols = pl.ds(j * LANE, LANE)
        return pltpu.make_async_copy(wq_hbm.at[:, cols], wq_v.at[0, :, cols],
                                     sems.at[S_WQ0 + j])

    def cp_wq(g):
        return pltpu.make_async_copy(wq_hbm.at[:, pl.ds(g * G, G)], wq_v.at[g],
                                     sems.at[S_WQ + g])

    def cp_wo(g):
        return pltpu.make_async_copy(wo_hbm.at[pl.ds(g * G, G), :], wo_v.at[g],
                                     sems.at[S_WO + g])

    def cp_k(g):
        return pltpu.make_async_copy(k_hbm.at[:, g], k_v.at[g], sems.at[S_K + g])

    def cp_v(g):
        return pltpu.make_async_copy(v_hbm.at[:, g], v_v.at[g], sems.at[S_V + g])

    phase = functools.partial(_phase, B=B, Sq=Sq, rep=rep, Dh=Dh)
    q_bufs = (q0, q1)
    o_bufs = (o0, o1)

    def run(t, par, **kw):
        refs = (x_v, wq_v, q_bufs[par], k_v, v_v, q_bufs[1 - par], o_bufs[1 - par],
                o_bufs[par], wo_v, acc_ref, outb, out_hbm, sems, S_OUT)
        phase(refs, t, **kw)

    def waits(t):
        static = isinstance(t, int)
        if not static or t < Hkv:
            cp_wq(t).wait()
        if not static or t <= Hkv:
            cp_k(t - 1).wait()
            cp_v(t - 1).wait()
        if not static or t >= 2:
            cp_wo(t - 2).wait()

    full = dict(do_a=True, do_b=True, do_c=True, final=False)
    n_mid = (Hkv - 4) // 2

    @pl.when(s == 0)
    def _():
        cp_x(0).start()
        cp_wq0(0).start()
        cp_x(1).start()
        for j in range(1, na):
            cp_wq0(j).start()
        for g in range(Hkv):
            cp_k(g).start()
            cp_v(g).start()
            if g + 1 < Hkv:
                cp_wq(g + 1).start()
            cp_wo(g).start()
        acc_ref[...] = jnp.zeros(acc_ref.shape, acc_ref.dtype)

        lo, hi, al = slice(0, M // 2), slice(M // 2, M), slice(0, M)
        steps = (
            ((cp_x(0), cp_wq0(0)), ((lo, 0),)),
            ((cp_x(1), cp_wq0(1)), ((hi, 0), (al, 1))),
            (tuple(cp_wq0(j) for j in range(2, na)),
             tuple((al, j) for j in range(2, na))),
        )
        for copies, pieces in steps:
            for c in copies:
                c.wait()
            for rows, j in pieces:
                sl = slice(j * LANE, (j + 1) * LANE)
                q0[rows, sl] = jnp.dot(
                    x_v[rows, :], wq_v[0, :, sl],
                    preferred_element_type=jnp.float32).astype(q0.dtype)

        waits(1)
        run(1, 1, do_a=True, do_b=True, do_c=False, final=False)
        waits(2)
        run(2, 0, **full)

    @pl.when(jnp.logical_and(s >= 1, s <= n_mid))
    def _():
        t = 2 * s + 1
        waits(t)
        waits(t + 1)
        run(t, 1, **full)
        run(t + 1, 0, **full)

    @pl.when(s == n_mid + 1)
    def _():
        for t in (Hkv - 1, Hkv, Hkv + 1):
            waits(t)
        run(Hkv - 1, 1, **full)
        run(Hkv, 0, do_a=False, do_b=True, do_c=True, final=False)
        run(Hkv + 1, 1, do_a=False, do_b=False, do_c=True, final=True)
        for j in range(nout):
            sl = slice(j * LANE, (j + 1) * LANE)
            pltpu.make_async_copy(outb.at[:, sl], out_hbm.at[:, sl],
                                  sems.at[S_OUT + j]).wait()


@jax.jit
def pallas_standalone__gqa_block_cached__near_ridge_kernel(
    x: jax.Array,
    k_cache: jax.Array,
    v_cache: jax.Array,
    wq: jax.Array,
    wo: jax.Array,
):
    B, Sq, D = x.shape
    _, Hkv, Sk, Dh = k_cache.shape
    Hq = wq.shape[1] // Dh
    rep = Hq // Hkv
    M = B * Sq
    G = rep * Dh
    assert Hkv % 2 == 0 and Hkv >= 4 and M % 2 == 0
    assert G % LANE == 0 and D % LANE == 0 and G // LANE >= 2

    x2 = x.reshape(M, D)

    kernel = functools.partial(_kernel, B=B, Sq=Sq, rep=rep, Dh=Dh, Hkv=Hkv)
    any_spec = pl.BlockSpec(memory_space=pl.ANY)
    n_sem = 2 + (G // LANE - 1) + 4 * Hkv + D // LANE
    out = pl.pallas_call(
        kernel,
        grid=((Hkv - 4) // 2 + 2,),
        in_specs=[any_spec] * 5,
        out_specs=any_spec,
        out_shape=jax.ShapeDtypeStruct((M, D), x.dtype),
        scratch_shapes=[
            pltpu.VMEM((M, D), x.dtype),
            pltpu.VMEM((Hkv, B, Sk, Dh), k_cache.dtype),
            pltpu.VMEM((Hkv, B, Sk, Dh), v_cache.dtype),
            pltpu.VMEM((Hkv, D, G), wq.dtype),
            pltpu.VMEM((Hkv, G, D), wo.dtype),
            pltpu.VMEM((M, G), x.dtype),
            pltpu.VMEM((M, G), x.dtype),
            pltpu.VMEM((M, G), x.dtype),
            pltpu.VMEM((M, G), x.dtype),
            pltpu.VMEM((M, D), jnp.float32),
            pltpu.VMEM((M, D), x.dtype),
            pltpu.SemaphoreType.DMA((n_sem,)),
        ],
        compiler_params=pltpu.CompilerParams(
            dimension_semantics=("arbitrary",),
            vmem_limit_bytes=64 * 1024 * 1024,
        ),
    )(x2, k_cache, v_cache, wq, wo)
    return out.reshape(B, Sq, D)
```
